```python
import os as _os
_os.environ.setdefault("JAX_PLATFORMS", "cpu")
import jax
import jax.numpy as jnp

def _softmax(x, axis=-1):
    return jax.nn.softmax(x, axis=axis)
def _gelu(x):
    return jax.nn.gelu(x, approximate=True)
def _silu(x):
    return jax.nn.silu(x)
def _sigmoid(x):
    return jax.nn.sigmoid(x)
def _layernorm(x, axis=-1, eps=1e-5):
    m = jnp.mean(x, axis=axis, keepdims=True)
    v = jnp.var(x, axis=axis, keepdims=True)
    return (x - m) / jnp.sqrt(v + eps)
def _scatter_add(tgt, idx, src, axis=0):
    return tgt.at[idx].add(src)
def _segment_sum(src, seg, n):
    return jax.ops.segment_sum(src, seg, n)
class _Rng:
    def __init__(self, key):
        self._k = key
    def _next(self):
        self._k, sub = jax.random.split(self._k)
        return sub
    def normal(self, shape):
        return jax.random.normal(self._next(), shape, dtype=jnp.bfloat16)
    def randint(self, lo, hi, shape):
        return jax.random.randint(self._next(), shape, lo, hi, dtype=jnp.int32)
    def uniform(self, shape, lo=0.0, hi=1.0):
        return jax.random.uniform(self._next(), shape, jnp.bfloat16, lo, hi)
    def permutation(self, n):
        return jax.random.permutation(self._next(), n)


kernel_name = 'concat_heads__softmax_full_mha__grouped_kv_mqa__prompt'

def setup_inputs():
    _rng = _Rng(jax.random.key(int.from_bytes(__import__("os").urandom(4), "little")))
    _w = (lambda a: (lambda t: t.astype(jnp.bfloat16) if jnp.issubdtype(t.dtype, jnp.floating) else t)(jnp.asarray(a)))
    def _A_setup():
        B, S, D = 1, 2048, 640
        return {
            "x": _w((lambda *s: _rng.normal(s) * 0.1)(B, S, D)),
            "wqkv": _w((lambda *s: _rng.normal(s) * 0.1)(D, 3 * D)),
            "wo": _w((lambda *s: _rng.normal(s) * 0.05)(D, D)),
        }
    _A_in = _A_setup()

    def _B_setup():
        B, S, D, H = 1, 2048, 640, 32
        Dh = D // H
        return {
            "x": _w((lambda *s: _rng.normal(s) * 0.05)(B, S, D)),
            "wq": _w((lambda *s: _rng.normal(s) * 0.4)(D, H * Dh)),
            "wk": _w((lambda *s: _rng.normal(s) * 0.4)(D, Dh)),
            "wv": _w((lambda *s: _rng.normal(s) * 0.05)(D, Dh)),
            "wo": _w((lambda *s: _rng.normal(s) * 0.05)(H * Dh, D)),
        }
    _B_in = _B_setup()

    return {
        "A_x": _A_in["x"],
        "A_wqkv": _A_in["wqkv"],
        "A_wo": _A_in["wo"],
        "B_x": _B_in["x"],
        "B_wq": _B_in["wq"],
        "B_wk": _B_in["wk"],
        "B_wv": _B_in["wv"],
        "B_wo": _B_in["wo"],
    }

def reference(A_x, A_wqkv, A_wo, B_x, B_wq, B_wk, B_wv, B_wo):
    def _A_ref(x, wqkv, wo):
        B, S, D = x.shape
        H = 32; Dh = D // H
        qkv = (lambda x, *d: x.transpose(*d))((x @ wqkv).reshape(B, S, 3, H, Dh), 2, 0, 3, 1, 4)
        q, k, v = qkv[0], qkv[1], qkv[2]
        scale = Dh ** -0.5
        scores = jnp.einsum("bhqd,bhkd->bhqk", q, k) * scale
        p = _softmax(scores, axis=-1)
        o = jnp.einsum("bhqk,bhkd->bhqd", p, v)
        return (lambda x, *d: x.transpose(*d))(o, 0, 2, 1, 3).reshape(B, S, D) @ wo

    def _B_ref(x, wq, wk, wv, wo):
        B, S, D = x.shape
        H = 32
        Dh = D // H
        q = (lambda x, *d: x.transpose(*d))((x @ wq).reshape(B, S, H, Dh), 0, 2, 1, 3)
        k = x @ wk
        v = x @ wv
        scores = jnp.einsum("bhqd,bkd->bhqk", q, k) * (Dh ** -0.5)
        p = _softmax(scores, axis=-1)
        o = jnp.einsum("bhqk,bkd->bhqd", p, v)
        return (lambda x, *d: x.transpose(*d))(o, 0, 2, 1, 3).reshape(B, S, H * Dh) @ wo

    a = _A_ref(A_x, A_wqkv, A_wo)
    b = _B_ref(B_x, B_wq, B_wk, B_wv, B_wo)
    return jnp.concatenate([a, b], axis=-1)
```

```python
import math

import jax
import jax.numpy as jnp
from jax import lax
import jax.experimental.pallas as pl
import jax.experimental.pallas.tpu as pltpu

S = 2048
D = 640
H = 32
DH = 20
HPG = 6
NG = 6
VR = 24
TQ = 512
NQ = S // TQ
CK = 128
NCK = S // CK
PC = 512

_F32 = jnp.float32
_BF16 = jnp.bfloat16
_NT = (((1,), (1,)), ((), ()))


def _kernel(xa_ref, xb_ref, wka_ref, wqva_ref, wkb_ref, wqvb_ref, woa_ref, wob_ref,
            out_ref, k_ref, qt_ref, vt_ref, ot_ref, s_ref, m_ref):
    qscale = (DH ** -0.5) * math.log2(math.e)

    def proj(c, carry):
        rows = pl.ds(pl.multiple_of(c * PC, PC), PC)
        xa = xa_ref[rows, :]
        xb = xb_ref[rows, :]
        ka = jnp.dot(xa, wka_ref[...], preferred_element_type=_F32).astype(_BF16)
        for g in range(NG):
            k_ref[g, rows, :] = ka[:, g * 128:(g + 1) * 128]
        k_ref[NG, rows, :] = jnp.dot(xb, wkb_ref[...], preferred_element_type=_F32).astype(_BF16)

        qva = lax.dot_general(wqva_ref[...], xa, _NT, preferred_element_type=_F32)
        qt_ref[0:NG, :, rows] = (qva[:NG * 128] * qscale).astype(_BF16).reshape(NG, 128, PC)
        va = qva[NG * 128:].reshape(H, VR, PC)
        r = lax.broadcasted_iota(jnp.int32, va.shape, 1)
        vt_ref[0:H, :, rows] = jnp.where(r == DH, 1.0, va)

        qvb = lax.dot_general(wqvb_ref[...], xb, _NT, preferred_element_type=_F32)
        qt_ref[NG:2 * NG, :, rows] = (qvb[:NG * 128] * qscale).astype(_BF16).reshape(NG, 128, PC)
        vb = qvb[NG * 128:NG * 128 + VR]
        rb = lax.broadcasted_iota(jnp.int32, vb.shape, 0)
        vt_ref[H, :, rows] = jnp.where(rb == DH, 1.0, vb)
        return carry

    lax.fori_loop(0, S // PC, proj, 0)

    def head_idx(hh):
        br = hh // H
        h = hh - br * H
        g = h // HPG
        j = h - g * HPG
        kg = jnp.where(br == 0, g, NG)
        qg = br * NG + g
        vi = jnp.where(br == 0, h, H)
        return kg, qg, j, vi

    def unit(u, qk, pv):
        cols = pl.ds(u * TQ, TQ)
        s_buf = s_ref.at[u]
        m_buf = m_ref.at[u]
        if qk is not None:
            kg, qg, j = qk
            q = qt_ref[qg, :, cols]
            r = lax.broadcasted_iota(jnp.int32, q.shape, 0)
            lo = j * DH
            qm = jnp.where((r >= lo) & (r < lo + DH), q.astype(_F32), 0.0).astype(_BF16)
        if pv is not None:
            vi, hh = pv
            mcur = m_buf[...]
        mrun = None
        acc = None
        for c in range(NCK):
            sl = pl.ds(c * CK, CK)
            if pv is not None:
                sc = s_buf[sl, :].reshape(CK // 8, 8, TQ)
                p = jnp.exp2(sc - mcur[None]).reshape(CK, TQ)
                d = jnp.dot(vt_ref[vi, :, sl], p, preferred_element_type=_F32)
                acc = d if acc is None else acc + d
            if qk is not None:
                s = jnp.dot(k_ref[kg, sl, :], qm, preferred_element_type=_F32)
                s_buf[sl, :] = s
                cm = jnp.max(s.reshape(CK // 8, 8, TQ), axis=0)
                mrun = cm if mrun is None else jnp.maximum(mrun, cm)
        if qk is not None:
            m_buf[...] = jnp.broadcast_to(jnp.max(mrun, axis=0, keepdims=True), (8, TQ))
        if pv is not None:
            ot_ref[hh, :, cols] = acc / acc[DH:DH + 1, :]

    for u in range(NQ):
        unit(u, (0, 0, 0), None)

    def body(hh, carry):
        kg, qg, j, _ = head_idx(hh + 1)
        _, _, _, vi = head_idx(hh)
        for u in range(NQ):
            unit(u, (kg, qg, j), (vi, hh))
        return carry

    lax.fori_loop(0, 2 * H - 1, body, 0)

    for u in range(NQ):
        unit(u, None, (H, 2 * H - 1))

    def oproj(c, carry):
        rows = pl.ds(pl.multiple_of(c * PC, PC), PC)
        for br, wo_ref in enumerate((woa_ref, wob_ref)):
            ot = ot_ref[br * H:(br + 1) * H, :, rows].reshape(H * VR, PC)
            o = ot.T.astype(_BF16)
            res = jnp.dot(o, wo_ref[...], preferred_element_type=_F32)
            out_ref[rows, br * D:(br + 1) * D] = res.astype(out_ref.dtype)
        return carry

    lax.fori_loop(0, S // PC, oproj, 0)


def _group_cols(w):
    w = jnp.pad(w, ((0, 0), (0, NG * HPG * DH - H * DH)))
    w = w.reshape(D, NG, HPG * DH)
    w = jnp.pad(w, ((0, 0), (0, 0), (0, 128 - HPG * DH)))
    return w.reshape(D, NG * 128)


def _head_rows(w):
    n = w.shape[1]
    w = w.reshape(-1, DH, n)
    w = jnp.pad(w, ((0, 0), (0, VR - DH), (0, 0)))
    return w.reshape(-1, n)


@jax.jit
def pallas_concat_heads__softmax_full_mha__grouped_kv_mqa__prompt_kernel(
    A_x: jax.Array,
    A_wqkv: jax.Array,
    A_wo: jax.Array,
    B_x: jax.Array,
    B_wq: jax.Array,
    B_wk: jax.Array,
    B_wv: jax.Array,
    B_wo: jax.Array,
):
    xa = A_x.reshape(S, D)
    xb = B_x.reshape(S, D)
    wka = _group_cols(A_wqkv[:, D:2 * D])
    wqva = jnp.concatenate(
        [_group_cols(A_wqkv[:, :D]).T, _head_rows(A_wqkv[:, 2 * D:].T)], axis=0)
    wkb = jnp.pad(jnp.concatenate([B_wk] * HPG, axis=1), ((0, 0), (0, 128 - HPG * DH)))
    wqvb = jnp.concatenate(
        [_group_cols(B_wq).T, jnp.pad(B_wv.T, ((0, 32 - DH), (0, 0)))], axis=0)
    woa = _head_rows(A_wo)
    wob = _head_rows(B_wo)

    out = pl.pallas_call(
        _kernel,
        out_shape=jax.ShapeDtypeStruct((S, 2 * D), A_x.dtype),
        scratch_shapes=[
            pltpu.VMEM((NG + 1, S, 128), _BF16),
            pltpu.VMEM((2 * NG, 128, S), _BF16),
            pltpu.VMEM((H + 1, VR, S), _F32),
            pltpu.VMEM((2 * H, VR, S), _F32),
            pltpu.VMEM((NQ, S, TQ), _F32),
            pltpu.VMEM((NQ, 8, TQ), _F32),
        ],
        compiler_params=pltpu.CompilerParams(vmem_limit_bytes=100 * 1024 * 1024),
    )(xa, xb, wka, wqva, wkb, wqvb, woa, wob)
    return out.reshape(1, S, 2 * D)
```

```python
import math

import jax
import jax.numpy as jnp
from jax import lax
import jax.experimental.pallas as pl
import jax.experimental.pallas.tpu as pltpu

S = 2048
D = 640
H = 32
DH = 20
HPG = 6
GW = HPG * DH
NG = 6
VR = 24
TQ = 512
NQ = S // TQ
CK = 128
NCK = S // CK
PC = 512
NPC = S // PC
HB = 2
NT5 = D // 128

_F32 = jnp.float32
_BF16 = jnp.bfloat16
_NT = (((1,), (1,)), ((), ()))

WTA_ROWS = 2 * D
WTB_ROWS = D + 64


def _kernel(xa_hbm, wqkv_hbm, woa_hbm, xb_hbm, wqb_hbm, wkb_hbm, wvb_hbm, wob_hbm,
            out_hbm,
            xa_v, xb_v, wqkv_v, wqb_v, wkb_v, wvb_v, woa_v, wob_v, wta_ref, wtb_ref,
            k_ref, qt_ref, vt_ref, ot_ref, s_ref, m_ref, o_v, sems, osems):
    qscale = (DH ** -0.5) * math.log2(math.e)

    def rows_of(c):
        if isinstance(c, int):
            return pl.ds(c * PC, PC)
        return pl.ds(pl.multiple_of(c * PC, PC), PC)

    def cp(src, dst, i):
        return pltpu.make_async_copy(src, dst, sems.at[i])

    def cp_xb(c):
        return pltpu.make_async_copy(xb_hbm.at[rows_of(c)], xb_v.at[rows_of(c)], sems.at[7 + c])

    def cp_out(c, br):
        cols = pl.ds(br * D, D)
        return pltpu.make_async_copy(o_v.at[rows_of(c), cols], out_hbm.at[rows_of(c), cols],
                                     osems.at[2 * c + br])

    c_wqb = cp(wqb_hbm, wqb_v, 0)
    c_wkb = cp(wkb_hbm, wkb_v, 1)
    c_wvb = cp(wvb_hbm, wvb_v, 2)
    c_wqkv = cp(wqkv_hbm, wqkv_v, 3)

    def cp_xa(c):
        return pltpu.make_async_copy(xa_hbm.at[rows_of(c)], xa_v.at[rows_of(c)],
                                     sems.at[7 + NPC + c])

    c_woa = cp(woa_hbm, woa_v, 5)
    c_wob = cp(wob_hbm, wob_v, 6)

    c_wqb.start()
    c_wkb.start()
    c_wvb.start()
    cp_xb(0).start()
    c_wqb.wait()
    for c in range(1, NPC):
        cp_xb(c).start()
    c_wqkv.start()
    for c in range(NPC):
        cp_xa(c).start()
    c_wkb.wait()
    c_wvb.wait()

    def store_q(base, res, cols):
        for g in range(NG):
            hi = min(g * GW + 128, res.shape[0])
            q = res[g * GW:hi] * qscale
            if hi - g * GW < 128:
                q = jnp.concatenate([q, jnp.zeros((128 - (hi - g * GW), PC), _F32)], axis=0)
            qt_ref[base + g, :, cols] = q.astype(_BF16)

    def unit(slot, cols, qk, pv, extra=None):
        s_buf = s_ref.at[slot]
        m_buf = m_ref.at[slot]
        if qk is not None:
            kg, qg, j = qk
            q = qt_ref[qg, :, cols]
            r = lax.broadcasted_iota(jnp.int32, q.shape, 0)
            lo = j * DH
            qm = jnp.where((r >= lo) & (r < lo + DH), q.astype(_F32), 0.0).astype(_BF16)
        if pv is not None:
            vi, hh = pv
            mcur = m_buf[...]
        mrun = None
        acc = None
        for c in range(NCK):
            sl = pl.ds(c * CK, CK)
            if pv is not None:
                sc = s_buf[sl, :].reshape(CK // 8, 8, TQ)
                p = jnp.exp2(sc - mcur[None]).reshape(CK, TQ)
                d = jnp.dot(vt_ref[vi, :, sl], p, preferred_element_type=_F32)
                acc = d if acc is None else acc + d
            if extra is not None:
                extra(c)
            if qk is not None:
                s = jnp.dot(k_ref[kg, sl, :], qm, preferred_element_type=_F32)
                s_buf[sl, :] = s
                cm = jnp.max(s.reshape(CK // 8, 8, TQ), axis=0)
                mrun = cm if mrun is None else jnp.maximum(mrun, cm)
        if qk is not None:
            m_buf[...] = jnp.broadcast_to(jnp.max(mrun, axis=0, keepdims=True), (8, TQ))
        if pv is not None:
            ot_ref[hh, :, cols] = acc / acc[DH:DH + 1, :]

    wtb_ref[0:D, :] = wqb_v[...].T
    zpad = jnp.zeros((32 - DH, D), _F32)
    wtb_ref[D:WTB_ROWS, :] = jnp.concatenate(
        [wvb_v[...].astype(_F32), zpad, wkb_v[...].astype(_F32), zpad], axis=0).astype(_BF16)

    def proj_b(c, carry):
        rows = rows_of(c)
        cp_xb(c).wait()
        res = lax.dot_general(wtb_ref[...], xb_v[rows, :], _NT, preferred_element_type=_F32)
        store_q(0, res, rows)
        vb = res[D:D + VR]
        rb = lax.broadcasted_iota(jnp.int32, vb.shape, 0)
        vt_ref[0, :, rows] = jnp.where(rb == DH, 1.0, vb)
        kt = res[D + 32:D + 32 + DH]
        kt = jnp.concatenate([kt] * HPG + [jnp.zeros((128 - GW, PC), _F32)], axis=0)
        k_ref[0, rows, :] = kt.T.astype(_BF16)
        return carry

    lax.fori_loop(0, NPC - 1, proj_b, 0)
    c_wqkv.wait()
    c_woa.start()
    c_wob.start()
    proj_b(NPC - 1, 0)
    wta_ref[0:D, :] = wqkv_v[:, 0:D].T
    wta_ref[D:2 * D, :] = wqkv_v[:, 2 * D:3 * D].T

    def proj_a(c, carry):
        rows = rows_of(c)
        cp_xa(c).wait()
        for b in range(HB):
            unit(b * NQ + c, rows, (0, 0, b), None)
        xa = xa_v[rows, :]
        ka = jnp.dot(xa, wqkv_v[:, D:2 * D], preferred_element_type=_F32)
        ka = jnp.concatenate([ka, jnp.zeros((PC, 128), _F32)], axis=1)
        for g in range(NG):
            k_ref[1 + g, rows, :] = ka[:, g * GW:g * GW + 128].astype(_BF16)
        res = lax.dot_general(wta_ref[...], xa, _NT, preferred_element_type=_F32)
        store_q(NG, res, rows)
        res = jnp.concatenate([res[D:], jnp.zeros((8, PC), _F32)], axis=0)
        r = lax.broadcasted_iota(jnp.int32, (VR, PC), 0)
        for h in range(H):
            vt_ref[1 + h, :, rows] = jnp.where(r == DH, 1.0, res[h * DH:h * DH + VR])
        return carry

    lax.fori_loop(0, NPC, proj_a, 0)

    def body(i, carry):
        kg, qg, j = carry
        hh = i * HB
        for b in range(HB):
            vi = jnp.maximum(hh + b - (H - 1), 0)
            for u in range(NQ):
                unit(b * NQ + u, pl.ds(u * TQ, TQ), (kg, qg, j + b), (vi, hh + b))
        switch = i + 2 == H // HB
        wrap = jnp.logical_or(j + HB == HPG, switch)
        j2 = jnp.where(wrap, 0, j + HB)
        qg2 = jnp.where(wrap, qg + 1, qg)
        kg2 = jnp.maximum(qg2 - (NG - 1), 0)
        return kg2, qg2, j2

    lax.fori_loop(0, 2 * H // HB - 1, body,
                  (jnp.int32(0), jnp.int32(0), jnp.int32(HB)))

    c_woa.wait()
    c_wob.wait()

    def o_cols(base, rows, lo, hi):
        parts = []
        for h in range(H):
            a, b = max(lo, h * DH), min(hi, (h + 1) * DH)
            if a < b:
                parts.append(ot_ref[base + h, a - h * DH:b - h * DH, rows])
        return jnp.concatenate(parts, axis=0).T.astype(_BF16)

    def oproj(c, carry):
        rows = rows_of(c)
        ob = o_cols(0, rows, 0, D)
        oa = o_cols(H, rows, 0, D - 128)
        tasks = [(1, n, k) for n in range(NT5) for k in range(NT5)]
        tasks += [(0, n, k) for n in range(NT5) for k in range(NT5 - 1)]
        accs = {}

        def run(br, n, k, o):
            wo_v = wob_v if br else woa_v
            d = jnp.dot(o, wo_v[k * 128:(k + 1) * 128, n * 128:(n + 1) * 128],
                        preferred_element_type=_F32)
            accs[br, n] = d if k == 0 else accs[br, n] + d
            if k == NT5 - 1:
                o_v[rows, br * D + n * 128:br * D + (n + 1) * 128] = (
                    accs.pop((br, n)).astype(o_v.dtype))
                if n == NT5 - 1:
                    cp_out(c, br).start()

        def piece(_):
            if tasks:
                br, n, k = tasks.pop(0)
                run(br, n, k, (ob if br else oa)[:, k * 128:(k + 1) * 128])

        for b in range(HB):
            unit(b * NQ + c, rows, None, (H - HB + 1 + b, 2 * H - HB + b), extra=piece)
        while tasks:
            piece(0)
        ol = o_cols(H, rows, D - 128, D)
        for n in range(NT5):
            run(0, n, NT5 - 1, ol)
        return carry

    lax.fori_loop(0, NPC, oproj, 0)
    for c in range(NPC):
        for br in range(2):
            cp_out(c, br).wait()


@jax.jit
def pallas_concat_heads__softmax_full_mha__grouped_kv_mqa__prompt_kernel(
    A_x: jax.Array,
    A_wqkv: jax.Array,
    A_wo: jax.Array,
    B_x: jax.Array,
    B_wq: jax.Array,
    B_wk: jax.Array,
    B_wv: jax.Array,
    B_wo: jax.Array,
):
    any_spec = pl.BlockSpec(memory_space=pl.ANY)
    out = pl.pallas_call(
        _kernel,
        out_shape=jax.ShapeDtypeStruct((S, 2 * D), A_x.dtype),
        in_specs=[any_spec] * 8,
        out_specs=any_spec,
        scratch_shapes=[
            pltpu.VMEM((S, D), _BF16),
            pltpu.VMEM((S, D), _BF16),
            pltpu.VMEM((D, 3 * D), _BF16),
            pltpu.VMEM((D, D), _BF16),
            pltpu.VMEM((DH, D), _BF16),
            pltpu.VMEM((DH, D), _BF16),
            pltpu.VMEM((D, D), _BF16),
            pltpu.VMEM((D, D), _BF16),
            pltpu.VMEM((WTA_ROWS, D), _BF16),
            pltpu.VMEM((WTB_ROWS, D), _BF16),
            pltpu.VMEM((NG + 1, S, 128), _BF16),
            pltpu.VMEM((2 * NG, 128, S), _BF16),
            pltpu.VMEM((H + 1, VR, S), _F32),
            pltpu.VMEM((2 * H, VR, S), _F32),
            pltpu.VMEM((HB * NQ, S, TQ), _F32),
            pltpu.VMEM((HB * NQ, 8, TQ), _F32),
            pltpu.VMEM((S, 2 * D), _BF16),
            pltpu.SemaphoreType.DMA((7 + 2 * NPC,)),
            pltpu.SemaphoreType.DMA((2 * NPC,)),
        ],
        compiler_params=pltpu.CompilerParams(vmem_limit_bytes=110 * 1024 * 1024),
    )(A_x.reshape(S, D), A_wqkv, A_wo, B_x.reshape(S, D), B_wq, B_wk.T, B_wv.T, B_wo)
    return out.reshape(1, S, 2 * D)
```

```python
import math

import jax
import jax.numpy as jnp
from jax import lax
import jax.experimental.pallas as pl
import jax.experimental.pallas.tpu as pltpu

S = 2048
D = 640
H = 32
DH = 20
NP = H // 2
VR = 24
TQ = 512
NQ = S // TQ
CK = 128
NCK = S // CK
PC = 512
NPC = S // PC
HB = 2
NT5 = D // 128
HPG = 6
GW = HPG * DH
NG = 6

_F32 = jnp.float32
_BF16 = jnp.bfloat16
_I32 = jnp.int32
_I8 = jnp.int8
_NT = (((1,), (1,)), ((), ()))

WTB_ROWS = D + 32 + 48

N1 = 14.0
W1 = 243.0
LAM = W1 * N1 * N1
MAGIC = 1.5 * 2.0 ** 23
TINY = 1e-30
FLAG_THR = 0.5
EQ_BOUND = DH * 0.5 * (14.0 + 8.0) + DH * 0.25
TAU0 = 2.0 ** -8 * math.log2(math.e)
TAU1 = 2.5 * 2.0 ** -8


def _limbs(t):
    u1 = t + MAGIC
    ih = u1 - MAGIC
    rl = t - ih
    u3 = rl * (W1 ** 0.5) + MAGIC
    bits = lambda v: lax.bitcast_convert_type(v, _I32)
    err = jnp.abs(ih) + jnp.abs(u3 - MAGIC)
    return bits(ih * 9.0 + MAGIC), bits(u1), bits(rl * W1 + MAGIC), bits(u3), err


def _low_half(shape):
    return lax.broadcasted_iota(_I32, shape, 1) < 4


def _assemble(l0, b3, b4, l3):
    shp = l0[:, 2].shape
    sub = _low_half(shp)
    h0, h3, h4, h5 = l0[:, 2], b3[:, 2], b4[:, 2], l3[:, 2]
    r0, r3, r4, r5 = [pltpu.roll(w, 4, 1) for w in (h0, h3, h4, h5)]
    z = jnp.zeros(shp, l0.dtype)

    def full(i, j):
        return [l0[:, i], l0[:, j]] * 3 + [b3[:, i], b3[:, j], b4[:, i], b4[:, j],
                                           l3[:, i], l3[:, j]]

    a = full(0, 1) + [jnp.where(sub, h0, r0), jnp.where(sub, h0, r3), jnp.where(sub, h4, r5), z]
    b = full(3, 4) + [jnp.where(sub, r0, h0), jnp.where(sub, r0, h3), jnp.where(sub, r4, h5), z]
    return jnp.concatenate(a, axis=1), jnp.concatenate(b, axis=1)


def _pair_reduce(v, op, red):
    sub = _low_half(v[:, 2].shape)
    a = op(op(v[:, 0], v[:, 1]), jnp.where(sub, v[:, 2], 0.0))
    b = op(op(v[:, 3], v[:, 4]), jnp.where(sub, 0.0, v[:, 2]))
    return red(a, axis=1, keepdims=True), red(b, axis=1, keepdims=True)


def _pair_rows(a, b):
    return jnp.stack([a, a, jnp.where(_low_half(a.shape), a, b), b, b], axis=1)


def _kernel(xa_hbm, wqkv_hbm, woa_hbm, xb_hbm, wqb_hbm, wkb_hbm, wvb_hbm, wob_hbm,
            out_hbm,
            xa_v, xb_v, wqkv_v, wqb_v, wkb_v, wvb_v, woa_v, wob_v, wta_ref, wtb_ref,
            kl_ref, ql_ref, sq_ref, kst_ref, kmx_ref, kt_ref, vt_ref, ot_ref, s_ref, m_ref, flag_ref,
            zero_ref,
            o_v, sems, osems):
    qscale = (DH ** -0.5) * math.log2(math.e)
    KB0 = 0

    def rows_of(c):
        if isinstance(c, int):
            return pl.ds(c * PC, PC)
        return pl.ds(pl.multiple_of(c * PC, PC), PC)

    def cp(src, dst, i):
        return pltpu.make_async_copy(src, dst, sems.at[i])

    def cp_xb(c):
        return pltpu.make_async_copy(xb_hbm.at[rows_of(c)], xb_v.at[rows_of(c)], sems.at[6 + c])

    def cp_xa(c):
        return pltpu.make_async_copy(xa_hbm.at[rows_of(c)], xa_v.at[rows_of(c)],
                                     sems.at[6 + NPC + c])

    def cp_out(c, br):
        cols = pl.ds(br * D, D)
        return pltpu.make_async_copy(o_v.at[rows_of(c), cols], out_hbm.at[rows_of(c), cols],
                                     osems.at[2 * c + br])

    c_wqb = cp(wqb_hbm, wqb_v, 0)
    c_wkb = cp(wkb_hbm, wkb_v, 1)
    c_wvb = cp(wvb_hbm, wvb_v, 2)
    c_wqkv = cp(wqkv_hbm, wqkv_v, 3)
    c_woa = cp(woa_hbm, woa_v, 4)
    c_wob = cp(wob_hbm, wob_v, 5)

    c_wqb.start()
    c_wkb.start()
    c_wvb.start()
    cp_xb(0).start()
    c_wqb.wait()
    for c in range(1, NPC):
        cp_xb(c).start()
    c_wqkv.start()
    for c in range(NPC):
        cp_xa(c).start()
    c_wkb.wait()
    c_wvb.wait()

    flag_ref[...] = jnp.zeros_like(flag_ref)
    kmx_ref[...] = jnp.zeros_like(kmx_ref)
    zero_ref[...] = jnp.zeros_like(zero_ref)

    def lane_fold(v):
        out = v[..., 0:128]
        for t in range(1, v.shape[-1] // 128):
            out = jnp.maximum(out, v[..., t * 128:(t + 1) * 128])
        return out

    def quant_q(zget, pbase, cols):
        for p in range(NP):
            z = zget(p).reshape(1, 5, 8, PC)
            sa, sb = _pair_reduce(jnp.abs(z), jnp.maximum, jnp.max)
            sa = jnp.broadcast_to(jnp.maximum(sa, TINY), (1, 8, PC))
            sb = jnp.broadcast_to(jnp.maximum(sb, TINY), (1, 8, PC))
            l0, l1, l2, l3, _ = _limbs(z * _pair_rows(N1 / sa, N1 / sb))
            qa, qb = _assemble(l0, l1, l2, l3)
            ql_ref[pbase + p, 0, :, cols] = qa[0].astype(_I8)
            ql_ref[pbase + p, 1, :, cols] = qb[0].astype(_I8)
            sq_ref[pbase + p, 0, :, cols] = sa[0]
            sq_ref[pbase + p, 1, :, cols] = sb[0]

    def track_kmax(kt, pbase, npairs):
        v = lane_fold(jnp.abs(kt)).reshape(npairs, 5, 8, 128)
        kmx_ref[pbase:pbase + npairs, 0:5] = jnp.maximum(kmx_ref[pbase:pbase + npairs, 0:5], v)

    def finish_kmax(pbase, npairs):
        sa, sb = _pair_reduce(kmx_ref[pbase:pbase + npairs, 0:5], jnp.maximum, jnp.max)
        for b, sc in enumerate((sa, sb)):
            sc = jnp.maximum(jnp.max(sc, axis=2, keepdims=True), TINY)
            kst_ref[pbase:pbase + npairs, b, 0] = jnp.broadcast_to(sc, (npairs, 8, 128))

    def quant_k(src, r0, pbase, npairs, rows):
        for p in range(npairs):
            pp = pbase + p
            z = src[r0 + p * 40:r0 + (p + 1) * 40, rows].reshape(1, 5, 8, PC)
            inv = _pair_rows(N1 / kst_ref[pp:pp + 1, 0, 0], N1 / kst_ref[pp:pp + 1, 1, 0])
            inv = jnp.concatenate([inv] * (PC // 128), axis=3)
            l0, l1, l2, l3, err = _limbs(z * inv)
            ka, kb = _assemble(l0, l2, l1, l3)
            kl_ref[pp, 0, rows, :] = ka[0].astype(jnp.int16).T.astype(_I8)
            kl_ref[pp, 1, rows, :] = kb[0].astype(jnp.int16).T.astype(_I8)
            ea, eb = _pair_reduce(err, jnp.add, jnp.sum)
            for b, e in enumerate((ea, eb)):
                e = jnp.broadcast_to(lane_fold(e), (1, 8, 128))
                kmx_ref[pp:pp + 1, 5 + b] = jnp.maximum(kmx_ref[pp:pp + 1, 5 + b], e)

    def finish_kerr(pbase, npairs):
        for b in range(2):
            e = jnp.max(kmx_ref[pbase:pbase + npairs, 5 + b], axis=2, keepdims=True)
            kst_ref[pbase:pbase + npairs, b, 1] = jnp.broadcast_to(
                0.5 * e + EQ_BOUND, (npairs, 8, 128))

    def unit(slot, cols, qk, pv, extra=None, seed_acc=False):
        s_buf = s_ref.at[slot]
        if qk is not None:
            kp, qp, b = qk
            q = ql_ref[qp, b, :, cols]
        if pv is not None:
            vi, hh = pv
            mcur = m_ref[slot, 0]
            ccur = m_ref[slot, 1]
        mrun = None
        acc = zero_ref[...] if seed_acc else None
        for c in range(NCK):
            sl = pl.ds(c * CK, CK)
            if pv is not None:
                sc = s_buf[sl, :].reshape(CK // 8, 8, TQ)
                p = jnp.exp2((sc - mcur[None]) * ccur[None]).reshape(CK, TQ)
                d = jnp.dot(vt_ref[vi, :, sl], p, preferred_element_type=_F32)
                acc = d if acc is None else acc + d
            if extra is not None:
                extra(c)
            if qk is not None:
                t = jnp.dot(kl_ref[kp, b, sl, :], q, preferred_element_type=_I32)
                s = t.astype(_F32)
                s_buf[sl, :] = s
                cm = jnp.max(s.reshape(CK // 8, 8, TQ), axis=0)
                mrun = cm if mrun is None else jnp.maximum(mrun, cm)
        if qk is not None:
            m = jnp.broadcast_to(jnp.max(mrun, axis=0, keepdims=True), (8, TQ))
            rep = lambda v: jnp.concatenate([v] * (TQ // 128), axis=1)
            cs = sq_ref[qp, b, :, cols] * rep(kst_ref[kp, b, 0] * (1.0 / LAM))
            m_ref[slot, 0] = m
            m_ref[slot, 1] = cs
            ok = rep(kst_ref[kp, b, 1]) * cs <= TAU0 + TAU1 * jnp.abs(m * cs)
            flag_ref[slot] = jnp.where(ok, flag_ref[slot], 1.0)
        if pv is not None:
            start = hh * VR if isinstance(hh, int) else pl.multiple_of(hh * VR, 8)
            ot_ref[pl.ds(start, VR), cols] = acc / acc[DH:DH + 1, :]

    wtb_ref[0:D, :] = wqb_v[...].T
    wk = wkb_v[...].astype(_F32)
    wtb_ref[D:WTB_ROWS, :] = jnp.concatenate(
        [wvb_v[...].astype(_F32), jnp.zeros((32 - DH, D), _F32), wk, wk,
         jnp.zeros((8, D), _F32)], axis=0).astype(_BF16)

    def proj_b(c, carry):
        rows = rows_of(c)
        cp_xb(c).wait()
        res = lax.dot_general(wtb_ref[...], xb_v[rows, :], _NT, preferred_element_type=_F32)
        quant_q(lambda p: res[p * 40:(p + 1) * 40] * qscale, 0, rows)
        vb = res[D:D + VR]
        rb = lax.broadcasted_iota(_I32, vb.shape, 0)
        vt_ref[0, :, rows] = jnp.where(rb == DH, 1.0, vb)
        kt = res[D + 32:D + 32 + 2 * DH]
        ot_ref[KB0:KB0 + 2 * DH, rows] = kt
        track_kmax(kt, 0, 1)
        return carry

    lax.fori_loop(0, NPC - 1, proj_b, 0)
    c_wqkv.wait()
    c_woa.start()
    c_wob.start()
    proj_b(NPC - 1, 0)
    for i in range(3):
        wta_ref[i * D:(i + 1) * D, :] = wqkv_v[:, i * D:(i + 1) * D].T
    finish_kmax(0, 1)

    def proj_k(c, carry):
        rows = rows_of(c)
        cp_xa(c).wait()
        quant_k(ot_ref, KB0, 0, 1, rows)
        kt = lax.dot_general(wta_ref[D:2 * D, :], xa_v[rows, :], _NT,
                             preferred_element_type=_F32)
        kt_ref[:, rows] = kt
        track_kmax(kt, 1, NP)
        return carry

    lax.fori_loop(0, NPC, proj_k, 0)
    finish_kmax(1, NP)
    finish_kerr(0, 1)

    def proj_a(c, carry):
        rows = rows_of(c)
        xa = xa_v[rows, :]
        quant_k(kt_ref, 0, 1, NP, rows)
        res = lax.dot_general(wta_ref[2 * D:3 * D, :], xa, _NT, preferred_element_type=_F32)
        res = jnp.concatenate([res, jnp.zeros((8, PC), _F32)], axis=0)
        r = lax.broadcasted_iota(_I32, (VR, PC), 0)
        for h in range(H):
            vt_ref[1 + h, :, rows] = jnp.where(r == DH, 1.0, res[h * DH:h * DH + VR])
        zq = lax.dot_general(wta_ref[0:D, :], xa, _NT, preferred_element_type=_F32)
        quant_q(lambda p: zq[p * 40:(p + 1) * 40] * qscale, NP, rows)
        for b in range(HB):
            unit(b * NQ + c, rows, (0, 0, b), None)
        return carry

    lax.fori_loop(0, NPC, proj_a, 0)
    finish_kerr(1, NP)

    def body(i, carry):
        qp = i + 1
        kp = jnp.maximum(qp - (NP - 1), 0)
        hh = i * HB
        for b in range(HB):
            vi = jnp.maximum(hh + b - (H - 1), 0)
            for u in range(NQ):
                unit(b * NQ + u, pl.ds(u * TQ, TQ), (kp, qp, b), (vi, hh + b),
                     seed_acc=(b, u) != (0, 0))
        return carry

    lax.fori_loop(0, 2 * NP - 1, body, 0)

    def fallback(k_ref, qt_ref):
        FC = 256

        def fproj(c, carry):
            rows = pl.ds(pl.multiple_of(c * FC, FC), FC)

            def store_q(base, res):
                res = jnp.concatenate([res[0:D] * qscale, jnp.zeros((128, FC), _F32)], axis=0)
                for g in range(NG):
                    qt_ref[base + g, :, rows] = res[g * GW:g * GW + 128].astype(_BF16)

            res = lax.dot_general(wtb_ref[...], xb_v[rows, :], _NT, preferred_element_type=_F32)
            store_q(0, res)
            kt = res[D + 32:D + 32 + 2 * DH]
            kt = jnp.concatenate([kt] * (HPG // 2) + [jnp.zeros((128 - GW, FC), _F32)], axis=0)
            k_ref[0, rows, :] = kt.T.astype(_BF16)
            store_q(NG, lax.dot_general(wta_ref[0:D, :], xa_v[rows, :], _NT,
                                        preferred_element_type=_F32))
            kt = jnp.concatenate([kt_ref[:, rows], jnp.zeros((128, FC), _F32)], axis=0)
            for g in range(NG):
                k_ref[1 + g, rows, :] = kt[g * GW:g * GW + 128].T.astype(_BF16)
            return carry

        lax.fori_loop(0, S // FC, fproj, 0)

        def fattn(t, carry):
            hh = t // NQ
            u = t - hh * NQ
            br = hh // H
            h = hh - br * H
            g = h // HPG
            lo = (h - g * HPG) * DH
            slot = (hh % HB) * NQ + u
            cols = rows_of(u)
            q = qt_ref[br * NG + g, :, cols]
            r = lax.broadcasted_iota(_I32, q.shape, 0)
            qm = jnp.where((r >= lo) & (r < lo + DH), q.astype(_F32), 0.0).astype(_BF16)

            def fqk(c, mrun):
                sl = pl.ds(pl.multiple_of(c * FC, FC), FC)
                sc = jnp.dot(k_ref[br * (1 + g), sl, :], qm, preferred_element_type=_F32)
                s_ref[slot, sl, :] = sc
                return jnp.maximum(mrun, jnp.max(sc.reshape(FC // 8, 8, TQ), axis=0))

            mrun = lax.fori_loop(0, S // FC, fqk, jnp.full((8, TQ), -jnp.inf, _F32))
            m_ref[slot, 0] = jnp.broadcast_to(jnp.max(mrun, axis=0, keepdims=True), (8, TQ))
            m_ref[slot, 1] = jnp.ones((8, TQ), _F32)

            @pl.when(hh < 2 * H - HB)
            def _():
                unit(slot, cols, None, (br * (1 + h), hh))

            return carry

        lax.fori_loop(0, 2 * H * NQ, fattn, 0)

    @pl.when(jnp.max(flag_ref[...]) > FLAG_THR)
    def _():
        pl.run_scoped(fallback,
                      pltpu.VMEM((NG + 1, S, 128), _BF16),
                      pltpu.VMEM((2 * NG, 128, S), _BF16))

    c_woa.wait()
    c_wob.wait()

    def o_cols(base, rows, lo, hi):
        parts = []
        for h in range(H):
            a, b = max(lo, h * DH), min(hi, (h + 1) * DH)
            if a < b:
                r0 = (base + h) * VR - h * DH
                parts.append(ot_ref[r0 + a:r0 + b, rows])
        return jnp.concatenate(parts, axis=0).T.astype(_BF16)

    def oproj(c, carry):
        rows = rows_of(c)
        ob = o_cols(0, rows, 0, D)
        oa = o_cols(H, rows, 0, D - 128)
        tasks = [(1, n, k) for n in range(NT5) for k in range(NT5)]
        tasks += [(0, n, k) for n in range(NT5) for k in range(NT5 - 1)]
        accs = {}

        def run(br, n, k, o):
            wo_v = wob_v if br else woa_v
            d = jnp.dot(o, wo_v[k * 128:(k + 1) * 128, n * 128:(n + 1) * 128],
                        preferred_element_type=_F32)
            accs[br, n] = d if k == 0 else accs[br, n] + d
            if k == NT5 - 1:
                o_v[rows, br * D + n * 128:br * D + (n + 1) * 128] = (
                    accs.pop((br, n)).astype(o_v.dtype))
                if n == NT5 - 1:
                    cp_out(c, br).start()

        def piece(_):
            if tasks:
                br, n, k = tasks.pop(0)
                run(br, n, k, (ob if br else oa)[:, k * 128:(k + 1) * 128])

        for b in range(HB):
            unit(b * NQ + c, rows, None, (H - HB + 1 + b, 2 * H - HB + b), extra=piece)
        while tasks:
            piece(0)
        ol = o_cols(H, rows, D - 128, D)
        for n in range(NT5):
            run(0, n, NT5 - 1, ol)
        return carry

    lax.fori_loop(0, NPC, oproj, 0)
    for c in range(NPC):
        for br in range(2):
            cp_out(c, br).wait()


@jax.jit
def pallas_concat_heads__softmax_full_mha__grouped_kv_mqa__prompt_kernel(
    A_x: jax.Array,
    A_wqkv: jax.Array,
    A_wo: jax.Array,
    B_x: jax.Array,
    B_wq: jax.Array,
    B_wk: jax.Array,
    B_wv: jax.Array,
    B_wo: jax.Array,
):
    any_spec = pl.BlockSpec(memory_space=pl.ANY)
    out = pl.pallas_call(
        _kernel,
        out_shape=jax.ShapeDtypeStruct((S, 2 * D), A_x.dtype),
        in_specs=[any_spec] * 8,
        out_specs=any_spec,
        scratch_shapes=[
            pltpu.VMEM((S, D), _BF16),
            pltpu.VMEM((S, D), _BF16),
            pltpu.VMEM((D, 3 * D), _BF16),
            pltpu.VMEM((D, D), _BF16),
            pltpu.VMEM((DH, D), _BF16),
            pltpu.VMEM((DH, D), _BF16),
            pltpu.VMEM((D, D), _BF16),
            pltpu.VMEM((D, D), _BF16),
            pltpu.VMEM((3 * D, D), _BF16),
            pltpu.VMEM((WTB_ROWS, D), _BF16),
            pltpu.VMEM((NP + 1, 2, S, 128), _I8),
            pltpu.VMEM((2 * NP, 2, 128, S), _I8),
            pltpu.VMEM((2 * NP, 2, 8, S), _F32),
            pltpu.VMEM((NP + 1, 2, 2, 8, 128), _F32),
            pltpu.VMEM((NP + 1, 7, 8, 128), _F32),
            pltpu.VMEM((D, S), _F32),
            pltpu.VMEM((H + 1, VR, S), _F32),
            pltpu.VMEM((2 * H * VR, S), _F32),
            pltpu.VMEM((HB * NQ, S, TQ), _F32),
            pltpu.VMEM((HB * NQ, 2, 8, TQ), _F32),
            pltpu.VMEM((HB * NQ, 8, TQ), _F32),
            pltpu.VMEM((VR, TQ), _F32),
            pltpu.VMEM((S, 2 * D), _BF16),
            pltpu.SemaphoreType.DMA((6 + 2 * NPC,)),
            pltpu.SemaphoreType.DMA((2 * NPC,)),
        ],
        compiler_params=pltpu.CompilerParams(vmem_limit_bytes=120 * 1024 * 1024),
    )(A_x.reshape(S, D), A_wqkv, A_wo, B_x.reshape(S, D), B_wq, B_wk.T, B_wv.T, B_wo)
    return out.reshape(1, S, 2 * D)
```

```python
import math

import jax
import jax.numpy as jnp
from jax import lax
import jax.experimental.pallas as pl
import jax.experimental.pallas.tpu as pltpu

S = 2048
D = 640
H = 32
DH = 20
NP = H // 2
PR = 2 * DH
VR = 24
TQ = 512
NQ = S // TQ
CK = 128
NCK = S // CK
PC = TQ
NPC = S // PC
HB = 2
NT5 = D // 128
HPG = 6
GW = HPG * DH
NG = 6
FC = 256

_F32 = jnp.float32
_BF16 = jnp.bfloat16
_I32 = jnp.int32
_I8 = jnp.int8
_NT = (((1,), (1,)), ((), ()))

WTB_V = D
WTB_K = D + 32
WTB_ROWS = D + 32 + 48

QSCALE = (DH ** -0.5) * math.log2(math.e)

N1 = 14.0
W1 = 243.0
LAM = W1 * N1 * N1
MAGIC = 1.5 * 2.0 ** 23
TINY = 1e-30
HUGE = 1e30
EQ_BOUND = DH * 0.5 * (14.0 + 8.0) + DH * 0.25
TAU0 = 2.0 ** -8 * math.log2(math.e)
TAU1 = 2.5 * 2.0 ** -8


def _limbs(t):
    u1 = t + MAGIC
    ih = u1 - MAGIC
    rl = t - ih
    u3 = rl * (W1 ** 0.5) + MAGIC
    bits = lambda v: lax.bitcast_convert_type(v, _I32)
    err = jnp.abs(ih) + jnp.abs(u3 - MAGIC)
    return bits(ih * 9.0 + MAGIC), bits(u1), bits(rl * W1 + MAGIC), bits(u3), err


def _recip(v):
    r = pl.reciprocal(v, approx=True)
    return r * (2.0 - v * r)


def _low_half(shape):
    return lax.broadcasted_iota(_I32, shape, 1) < 4


def _assemble(l0, b3, b4, l3):
    shp = l0[:, 2].shape
    sub = _low_half(shp)
    h0, h3, h4, h5 = l0[:, 2], b3[:, 2], b4[:, 2], l3[:, 2]
    r0, r3, r4, r5 = [pltpu.roll(w, 4, 1) for w in (h0, h3, h4, h5)]
    z = jnp.zeros(shp, l0.dtype)

    def full(i, j):
        return [l0[:, i], l0[:, j]] * 3 + [b3[:, i], b3[:, j], b4[:, i], b4[:, j],
                                           l3[:, i], l3[:, j]]

    a = full(0, 1) + [jnp.where(sub, h0, r0), jnp.where(sub, h0, r3), jnp.where(sub, h4, r5), z]
    b = full(3, 4) + [jnp.where(sub, r0, h0), jnp.where(sub, r0, h3), jnp.where(sub, r4, h5), z]
    return jnp.concatenate(a, axis=1), jnp.concatenate(b, axis=1)


def _pair_reduce(v, op, red):
    sub = _low_half(v[:, 2].shape)
    a = op(op(v[:, 0], v[:, 1]), jnp.where(sub, v[:, 2], 0.0))
    b = op(op(v[:, 3], v[:, 4]), jnp.where(sub, 0.0, v[:, 2]))
    return red(a, axis=1, keepdims=True), red(b, axis=1, keepdims=True)


def _pair_rows(a, b):
    return jnp.stack([a, a, jnp.where(_low_half(a.shape), a, b), b, b], axis=1)


def _lane_fold(v):
    out = v[..., 0:128]
    for t in range(1, v.shape[-1] // 128):
        out = jnp.maximum(out, v[..., t * 128:(t + 1) * 128])
    return out


def _kernel(xa_hbm, wqkv_hbm, woa_hbm, xb_hbm, wqb_hbm, wkb_hbm, wvb_hbm, wob_hbm,
            out_hbm,
            xa_v, xb_v, wqkv_v, wqb_v, wkb_v, wvb_v, woa_v, wob_v, wta_ref, wtb_ref,
            kl_ref, ql_ref, sq_ref, kst_ref, kmx_ref, kt_ref, vt_ref, ot_ref,
            s_ref, m_ref, flag_ref, zero_ref, o_v, sems, osems):

    def rows_of(c):
        if isinstance(c, int):
            return pl.ds(c * PC, PC)
        return pl.ds(pl.multiple_of(c * PC, PC), PC)

    def cp(src, dst, i):
        return pltpu.make_async_copy(src, dst, sems.at[i])

    def cp_xb(c):
        return cp(xb_hbm.at[rows_of(c)], xb_v.at[rows_of(c)], 6 + c)

    def cp_xa(c):
        return cp(xa_hbm.at[rows_of(c)], xa_v.at[rows_of(c)], 6 + NPC + c)

    def cp_out(c, br):
        cols = pl.ds(br * D, D)
        return pltpu.make_async_copy(o_v.at[rows_of(c), cols], out_hbm.at[rows_of(c), cols],
                                     osems.at[2 * c + br])

    c_wqb = cp(wqb_hbm, wqb_v, 0)
    c_wkb = cp(wkb_hbm, wkb_v, 1)
    c_wvb = cp(wvb_hbm, wvb_v, 2)
    c_wqkv = cp(wqkv_hbm, wqkv_v, 3)
    c_woa = cp(woa_hbm, woa_v, 4)
    c_wob = cp(wob_hbm, wob_v, 5)

    c_wqb.start()
    c_wkb.start()
    c_wvb.start()
    cp_xb(0).start()
    c_wqb.wait()
    for c in range(1, NPC):
        cp_xb(c).start()
    c_wqkv.start()
    for c in range(NPC):
        cp_xa(c).start()
    c_wkb.wait()
    c_wvb.wait()

    flag_ref[...] = jnp.zeros_like(flag_ref)
    kmx_ref[...] = jnp.zeros_like(kmx_ref)
    zero_ref[...] = jnp.zeros_like(zero_ref)

    def quant_q(zq, pbase, cols):
        for p in range(NP):
            z = zq[p * PR:(p + 1) * PR].reshape(1, 5, 8, PC)
            sa, sb = _pair_reduce(jnp.abs(z), jnp.maximum, jnp.max)
            sa = jnp.broadcast_to(jnp.maximum(sa, TINY), (1, 8, PC))
            sb = jnp.broadcast_to(jnp.maximum(sb, TINY), (1, 8, PC))
            l0, l1, l2, l3, _ = _limbs(z * _pair_rows(N1 * _recip(sa), N1 * _recip(sb)))
            qa, qb = _assemble(l0, l1, l2, l3)
            ql_ref[pbase + p, 0, :, cols] = qa[0].astype(_I8)
            ql_ref[pbase + p, 1, :, cols] = qb[0].astype(_I8)
            sq_ref[pbase + p, 0, :, cols] = sa[0]
            sq_ref[pbase + p, 1, :, cols] = sb[0]

    def track_kmax(kt, pbase, npairs):
        v = _lane_fold(jnp.abs(kt)).reshape(npairs, 5, 8, 128)
        kmx_ref[pbase:pbase + npairs, 0:5] = jnp.maximum(kmx_ref[pbase:pbase + npairs, 0:5], v)

    def finish_kmax(pbase, npairs):
        sa, sb = _pair_reduce(kmx_ref[pbase:pbase + npairs, 0:5], jnp.maximum, jnp.max)
        for b, sc in enumerate((sa, sb)):
            sc = jnp.maximum(jnp.max(sc, axis=2, keepdims=True), TINY)
            sc = jnp.broadcast_to(sc, (npairs, 8, 128))
            kst_ref[pbase:pbase + npairs, b, 0] = sc * (QSCALE / LAM)
            kst_ref[pbase:pbase + npairs, b, 2] = N1 / sc

    def quant_k(src, pbase, npairs, rows):
        for p in range(npairs):
            pp = pbase + p
            z = src[p * PR:(p + 1) * PR, rows].reshape(1, 5, 8, PC)
            inv = _pair_rows(kst_ref[pp:pp + 1, 0, 2], kst_ref[pp:pp + 1, 1, 2])
            inv = jnp.concatenate([inv] * (PC // 128), axis=3)
            l0, l1, l2, l3, err = _limbs(z * inv)
            ka, kb = _assemble(l0, l2, l1, l3)
            kl_ref[pp, 0, rows, :] = ka[0].astype(jnp.int16).T.astype(_I8)
            kl_ref[pp, 1, rows, :] = kb[0].astype(jnp.int16).T.astype(_I8)
            ea, eb = _pair_reduce(err, jnp.add, jnp.sum)
            for b, e in enumerate((ea, eb)):
                e = jnp.broadcast_to(_lane_fold(e), (1, 8, 128))
                kmx_ref[pp:pp + 1, 5 + b] = jnp.maximum(kmx_ref[pp:pp + 1, 5 + b], e)

    def finish_kerr(pbase, npairs):
        for b in range(2):
            e = jnp.max(kmx_ref[pbase:pbase + npairs, 5 + b], axis=2, keepdims=True)
            kst_ref[pbase:pbase + npairs, b, 1] = jnp.broadcast_to(
                0.5 * e + EQ_BOUND, (npairs, 8, 128))

    def unit(slot, cols, qk, pv, extra=None, seed_acc=False):
        s_buf = s_ref.at[slot]
        if qk is not None:
            kp, qp, b = qk
            q = ql_ref[qp, b, :, cols]
        if pv is not None:
            vi, hh = pv
            mcur = m_ref[slot, 0]
            ccur = m_ref[slot, 1]
        mrun = None
        acc = zero_ref[...] if seed_acc else None
        for c in range(NCK):
            sl = pl.ds(c * CK, CK)
            if pv is not None:
                sc = s_buf[sl, :].reshape(CK // 8, 8, TQ)
                p = jnp.exp2((sc - mcur[None]) * ccur[None]).reshape(CK, TQ)
                d = jnp.dot(vt_ref[vi, :, sl], p, preferred_element_type=_F32)
                acc = d if acc is None else acc + d
            if extra is not None:
                extra()
            if qk is not None:
                t = jnp.dot(kl_ref[kp, b, sl, :], q, preferred_element_type=_I32)
                s = t.astype(_F32)
                s_buf[sl, :] = s
                s3 = s.reshape(CK // 8, 8, TQ)
                for r in range(CK // 8):
                    mrun = s3[r] if mrun is None else jnp.maximum(mrun, s3[r])
        if qk is not None:
            m = jnp.broadcast_to(jnp.max(mrun, axis=0, keepdims=True), (8, TQ))
            rep = lambda v: jnp.concatenate([v] * (TQ // 128), axis=1)
            sq = sq_ref[qp, b, :, cols]
            sk = rep(kst_ref[kp, b, 0])
            cs = sq * sk
            m_ref[slot, 0] = m
            m_ref[slot, 1] = cs
            err = rep(kst_ref[kp, b, 1]) * cs
            ok = ((err <= TAU0 + TAU1 * jnp.abs(m * cs))
                  & (jnp.maximum(jnp.maximum(sq, sk), err) < HUGE))
            flag_ref[slot] = jnp.where(ok, flag_ref[slot], 1.0)
        if pv is not None:
            start = hh * VR if isinstance(hh, int) else pl.multiple_of(hh * VR, 8)
            ot_ref[pl.ds(start, VR), cols] = acc * _recip(acc[DH:DH + 1, :])

    wtb_ref[0:D, :] = wqb_v[...].T
    wk = wkb_v[...].astype(_F32)
    wtb_ref[WTB_V:WTB_ROWS, :] = jnp.concatenate(
        [wvb_v[...].astype(_F32), jnp.zeros((32 - DH, D), _F32), wk, wk,
         jnp.zeros((8, D), _F32)], axis=0).astype(_BF16)

    def proj_b(c, carry):
        rows = rows_of(c)
        cp_xb(c).wait()
        res = lax.dot_general(wtb_ref[...], xb_v[rows, :], _NT, preferred_element_type=_F32)
        quant_q(res, 0, rows)
        vb = res[WTB_V:WTB_V + VR]
        rb = lax.broadcasted_iota(_I32, vb.shape, 0)
        vt_ref[0, :, rows] = jnp.where(rb == DH, 1.0, vb)
        kt = res[WTB_K:WTB_K + PR]
        ot_ref[0:PR, rows] = kt
        track_kmax(kt, 0, 1)
        return carry

    lax.fori_loop(0, NPC - 1, proj_b, 0)
    c_wqkv.wait()
    c_woa.start()
    c_wob.start()
    proj_b(NPC - 1, 0)
    for i in range(3):
        wta_ref[i * D:(i + 1) * D, :] = wqkv_v[:, i * D:(i + 1) * D].T
    finish_kmax(0, 1)

    def proj_qk(c, carry):
        rows = rows_of(c)
        cp_xa(c).wait()
        quant_k(ot_ref, 0, 1, rows)
        xa = xa_v[rows, :]
        zq = lax.dot_general(wta_ref[0:D, :], xa, _NT, preferred_element_type=_F32)
        quant_q(zq, NP, rows)
        kt = lax.dot_general(wta_ref[D:2 * D, :], xa, _NT, preferred_element_type=_F32)
        kt_ref[:, rows] = kt
        track_kmax(kt, 1, NP)
        return carry

    lax.fori_loop(0, NPC, proj_qk, 0)
    finish_kmax(1, NP)
    finish_kerr(0, 1)

    def proj_v(c, carry):
        rows = rows_of(c)
        quant_k(kt_ref, 1, NP, rows)
        res = lax.dot_general(wta_ref[2 * D:3 * D, :], xa_v[rows, :], _NT,
                              preferred_element_type=_F32)
        res = jnp.concatenate([res, jnp.zeros((8, PC), _F32)], axis=0)
        r = lax.broadcasted_iota(_I32, (VR, PC), 0)
        for h in range(H):
            vt_ref[1 + h, :, rows] = jnp.where(r == DH, 1.0, res[h * DH:h * DH + VR])
        for b in range(HB):
            unit(b * NQ + c, rows, (0, 0, b), None)
        return carry

    lax.fori_loop(0, NPC, proj_v, 0)
    finish_kerr(1, NP)

    def body(i, carry):
        qp = i + 1
        kp = jnp.maximum(qp - (NP - 1), 0)
        hh = i * HB
        for b in range(HB):
            vi = jnp.maximum(hh + b - (H - 1), 0)
            for u in range(NQ):
                unit(b * NQ + u, pl.ds(u * TQ, TQ), (kp, qp, b), (vi, hh + b),
                     seed_acc=(b, u) != (0, 0))
        return carry

    lax.fori_loop(0, 2 * NP - 1, body, 0)

    def fallback(k_ref, qt_ref):
        def fproj(c, carry):
            rows = pl.ds(pl.multiple_of(c * FC, FC), FC)

            def store_q(base, res):
                res = jnp.concatenate([res[0:D] * QSCALE, jnp.zeros((128, FC), _F32)], axis=0)
                for g in range(NG):
                    qt_ref[base + g, :, rows] = res[g * GW:g * GW + 128].astype(_BF16)

            res = lax.dot_general(wtb_ref[...], xb_v[rows, :], _NT, preferred_element_type=_F32)
            store_q(0, res)
            kt = res[WTB_K:WTB_K + PR]
            kt = jnp.concatenate([kt] * (HPG // 2) + [jnp.zeros((128 - GW, FC), _F32)], axis=0)
            k_ref[0, rows, :] = kt.T.astype(_BF16)
            store_q(NG, lax.dot_general(wta_ref[0:D, :], xa_v[rows, :], _NT,
                                        preferred_element_type=_F32))
            kt = jnp.concatenate([kt_ref[:, rows], jnp.zeros((128, FC), _F32)], axis=0)
            for g in range(NG):
                k_ref[1 + g, rows, :] = kt[g * GW:g * GW + 128].T.astype(_BF16)
            return carry

        lax.fori_loop(0, S // FC, fproj, 0)

        def fattn(t, carry):
            hh = t // NQ
            u = t - hh * NQ
            br = hh // H
            h = hh - br * H
            g = h // HPG
            lo = (h - g * HPG) * DH
            slot = (hh % HB) * NQ + u
            cols = rows_of(u)
            q = qt_ref[br * NG + g, :, cols]
            r = lax.broadcasted_iota(_I32, q.shape, 0)
            qm = jnp.where((r >= lo) & (r < lo + DH), q.astype(_F32), 0.0).astype(_BF16)

            def fqk(c, mrun):
                sl = pl.ds(pl.multiple_of(c * FC, FC), FC)
                sc = jnp.dot(k_ref[br * (1 + g), sl, :], qm, preferred_element_type=_F32)
                s_ref[slot, sl, :] = sc
                return jnp.maximum(mrun, jnp.max(sc.reshape(FC // 8, 8, TQ), axis=0))

            mrun = lax.fori_loop(0, S // FC, fqk, jnp.full((8, TQ), -jnp.inf, _F32))
            m_ref[slot, 0] = jnp.broadcast_to(jnp.max(mrun, axis=0, keepdims=True), (8, TQ))
            m_ref[slot, 1] = jnp.ones((8, TQ), _F32)

            @pl.when(hh < 2 * H - HB)
            def _():
                unit(slot, cols, None, (br * (1 + h), hh))

            return carry

        lax.fori_loop(0, 2 * H * NQ, fattn, 0)

    @pl.when(jnp.max(flag_ref[...]) > 0.5)
    def _():
        pl.run_scoped(fallback,
                      pltpu.VMEM((NG + 1, S, 128), _BF16),
                      pltpu.VMEM((2 * NG, 128, S), _BF16))

    c_woa.wait()
    c_wob.wait()

    def o_cols(base, rows, lo, hi):
        parts = []
        for h in range(H):
            a, b = max(lo, h * DH), min(hi, (h + 1) * DH)
            if a < b:
                r0 = (base + h) * VR - h * DH
                parts.append(ot_ref[r0 + a:r0 + b, rows])
        return jnp.concatenate(parts, axis=0).T.astype(_BF16)

    def oproj(c, carry):
        rows = rows_of(c)
        ob = o_cols(0, rows, 0, D)
        oa = o_cols(H, rows, 0, D - 128)
        tasks = [(1, n, k) for n in range(NT5) for k in range(NT5)]
        tasks += [(0, n, k) for n in range(NT5) for k in range(NT5 - 1)]
        accs = {}

        def run(br, n, k, o):
            wo_v = wob_v if br else woa_v
            d = jnp.dot(o, wo_v[k * 128:(k + 1) * 128, n * 128:(n + 1) * 128],
                        preferred_element_type=_F32)
            accs[br, n] = d if k == 0 else accs[br, n] + d
            if k == NT5 - 1:
                o_v[rows, br * D + n * 128:br * D + (n + 1) * 128] = (
                    accs.pop((br, n)).astype(o_v.dtype))
                if n == NT5 - 1:
                    cp_out(c, br).start()

        def piece():
            if tasks:
                br, n, k = tasks.pop(0)
                run(br, n, k, (ob if br else oa)[:, k * 128:(k + 1) * 128])

        for b in range(HB):
            unit(b * NQ + c, rows, None, (H - HB + 1 + b, 2 * H - HB + b), extra=piece)
        while tasks:
            piece()
        ol = o_cols(H, rows, D - 128, D)
        for n in range(NT5):
            run(0, n, NT5 - 1, ol)
        return carry

    lax.fori_loop(0, NPC, oproj, 0)
    for c in range(NPC):
        for br in range(2):
            cp_out(c, br).wait()


@jax.jit
def pallas_concat_heads__softmax_full_mha__grouped_kv_mqa__prompt_kernel(
    A_x: jax.Array,
    A_wqkv: jax.Array,
    A_wo: jax.Array,
    B_x: jax.Array,
    B_wq: jax.Array,
    B_wk: jax.Array,
    B_wv: jax.Array,
    B_wo: jax.Array,
):
    any_spec = pl.BlockSpec(memory_space=pl.ANY)
    out = pl.pallas_call(
        _kernel,
        out_shape=jax.ShapeDtypeStruct((S, 2 * D), A_x.dtype),
        in_specs=[any_spec] * 8,
        out_specs=any_spec,
        scratch_shapes=[
            pltpu.VMEM((S, D), _BF16),
            pltpu.VMEM((S, D), _BF16),
            pltpu.VMEM((D, 3 * D), _BF16),
            pltpu.VMEM((D, D), _BF16),
            pltpu.VMEM((DH, D), _BF16),
            pltpu.VMEM((DH, D), _BF16),
            pltpu.VMEM((D, D), _BF16),
            pltpu.VMEM((D, D), _BF16),
            pltpu.VMEM((3 * D, D), _BF16),
            pltpu.VMEM((WTB_ROWS, D), _BF16),
            pltpu.VMEM((NP + 1, 2, S, 128), _I8),
            pltpu.VMEM((2 * NP, 2, 128, S), _I8),
            pltpu.VMEM((2 * NP, 2, 8, S), _F32),
            pltpu.VMEM((NP + 1, 2, 3, 8, 128), _F32),
            pltpu.VMEM((NP + 1, 7, 8, 128), _F32),
            pltpu.VMEM((D, S), _F32),
            pltpu.VMEM((H + 1, VR, S), _F32),
            pltpu.VMEM((2 * H * VR, S), _F32),
            pltpu.VMEM((HB * NQ, S, TQ), _F32),
            pltpu.VMEM((HB * NQ, 2, 8, TQ), _F32),
            pltpu.VMEM((HB * NQ, 8, TQ), _F32),
            pltpu.VMEM((VR, TQ), _F32),
            pltpu.VMEM((S, 2 * D), _BF16),
            pltpu.SemaphoreType.DMA((6 + 2 * NPC,)),
            pltpu.SemaphoreType.DMA((2 * NPC,)),
        ],
        compiler_params=pltpu.CompilerParams(vmem_limit_bytes=120 * 1024 * 1024),
    )(A_x.reshape(S, D), A_wqkv, A_wo, B_x.reshape(S, D), B_wq, B_wk.T, B_wv.T, B_wo)
    return out.reshape(1, S, 2 * D)
```
